```python
import jax
import jax.numpy as jnp

def _softmax(x, axis=-1):
    return jax.nn.softmax(x, axis=axis)
def _gelu(x):
    return jax.nn.gelu(x, approximate=True)
def _silu(x):
    return jax.nn.silu(x)
def _sigmoid(x):
    return jax.nn.sigmoid(x)
def _layernorm(x, axis=-1, eps=1e-5):
    m = jnp.mean(x, axis=axis, keepdims=True)
    v = jnp.var(x, axis=axis, keepdims=True)
    return (x - m) / jnp.sqrt(v + eps)
def _scatter_add(tgt, idx, src, axis=0):
    return tgt.at[idx].add(src)
def _segment_sum(src, seg, n):
    return jax.ops.segment_sum(src, seg, n)
class _Rng:
    def __init__(self, key):
        self._k = key
    def _next(self):
        self._k, sub = jax.random.split(self._k)
        return sub
    def normal(self, shape):
        return jax.random.normal(self._next(), shape, dtype=jnp.bfloat16)
    def randint(self, lo, hi, shape):
        return jax.random.randint(self._next(), shape, lo, hi, dtype=jnp.int32)
    def uniform(self, shape, lo=0.0, hi=1.0):
        return jax.random.uniform(self._next(), shape, jnp.bfloat16, lo, hi)
    def permutation(self, n):
        return jax.random.permutation(self._next(), n)


kernel_name = 'gated_mix__mha_block_cached__moe_arch_mod__decode'

def setup_inputs():
    _rng = _Rng(jax.random.key(int.from_bytes(__import__("os").urandom(4), "little")))
    _w = (lambda a: (lambda t: t.astype(jnp.bfloat16) if jnp.issubdtype(t.dtype, jnp.floating) else t)(jnp.asarray(a)))
    def _A_setup():
        B, Sq, D = 4, 1, 1024
        H, Sk, Dh = 32, 8192, 128
        return {
            "x": _w((lambda *s: _rng.normal(s) * 0.05)(B, Sq, D)),
            "k_cache": _w((lambda *s: _rng.normal(s) * 0.05)(B, H, Sk, Dh)),
            "v_cache": _w((lambda *s: _rng.normal(s) * 0.05)(B, H, Sk, Dh)),
            "wq": _w((lambda *s: _rng.normal(s) * 0.05)(D, H * Dh) * (D ** -0.5)),
            "wo": _w((lambda *s: _rng.normal(s) * 0.05)(H * Dh, D) * ((H * Dh) ** -0.5)),
        }
    _A_in = _A_setup()

    def _B_setup():
        B, S, D, F, C = 4, 1, 1024, 3584, 1
        return {
            "x": _w((lambda *s: _rng.normal(s) * 0.05)(B, S, D)),
            "w_r": _w((lambda *s: _rng.normal(s) * 0.05)(D)),
            "w_gate": _w((lambda *s: _rng.normal(s) * 0.05)(D, F)),
            "w_up": _w((lambda *s: _rng.normal(s) * 0.05)(D, F)),
            "w_down": _w((lambda *s: _rng.normal(s) * 0.05)(F, D)),
        }
    _B_in = _B_setup()

    return {
        "A_x": _A_in["x"],
        "A_k_cache": _A_in["k_cache"],
        "A_v_cache": _A_in["v_cache"],
        "A_wq": _A_in["wq"],
        "A_wo": _A_in["wo"],
        "B_x": _B_in["x"],
        "B_w_r": _B_in["w_r"],
        "B_w_gate": _B_in["w_gate"],
        "B_w_up": _B_in["w_up"],
        "B_w_down": _B_in["w_down"],
        "gate_w": _w((lambda *s: _rng.normal(s) * 0.05)(1024)),
    }

def reference(A_x, A_k_cache, A_v_cache, A_wq, A_wo, B_x, B_w_r, B_w_gate, B_w_up, B_w_down, gate_w):
    def _A_ref(x, k_cache, v_cache, wq, wo):
        B, Sq, D = x.shape
        H, Dh = 32, 128
        q = (lambda x, *d: x.transpose(*d))((x @ wq).reshape(B, Sq, H, Dh), 0, 2, 1, 3)
        scores = jnp.einsum("bhqd,bhkd->bhqk", q, k_cache) * (Dh ** -0.5)
        p = _softmax(scores, axis=-1)
        o = jnp.einsum("bhqk,bhkd->bhqd", p, v_cache)
        return (lambda x, *d: x.transpose(*d))(o, 0, 2, 1, 3).reshape(B, Sq, H * Dh) @ wo

    def _B_ref(x, w_r, w_gate, w_up, w_down):
        B, S, D = x.shape
        C = 1
        r = x @ w_r
        idx = jnp.argsort(-r, axis=-1)[:, :C]
        idx_e = jnp.repeat(idx.reshape(B, C, 1), D, axis=2)
        x_sel = jnp.take_along_axis(x, idx_e, axis=1)
        g = _silu(x_sel @ w_gate)
        u = x_sel @ w_up
        y = (g * u) @ w_down
        r_sel = _sigmoid(jnp.take_along_axis(r, idx, axis=1))
        y = y * r_sel.reshape(B, C, 1)
        b_off = (jnp.arange(B) * S).reshape(B, 1)
        flat_idx = (idx + b_off).reshape(B * C)
        zero = (x * 0.0).reshape(B * S, D)
        upd = _scatter_add(zero, flat_idx, y.reshape(B * C, D), axis=0)
        return x + upd.reshape(B, S, D)

    x = A_x
    g = _sigmoid((x * gate_w).sum(-1, keepdims=True))
    a = _A_ref(x, A_k_cache, A_v_cache, A_wq, A_wo)
    b = _B_ref(x, B_w_r, B_w_gate, B_w_up, B_w_down)
    return g * a + (1 - g) * b
```

```python
import functools
import jax
import jax.numpy as jnp
import jax.experimental.pallas as pl
import jax.experimental.pallas.tpu as pltpu


def build(NR=4, NC=4, vmem_mb=64):
    B, D, H, Sk, Dh, F = 4, 1024, 32, 8192, 128, 3584
    CH = Sk // NC
    NF = F // 128
    NI = B * H
    scale = Dh ** -0.5
    f32, bf16 = jnp.float32, jnp.bfloat16

    def kern(ax_ref, k_hbm, v_hbm, wq_hbm, wo_hbm, wr_ref, wg_hbm, wu_hbm, wd_hbm, gw_ref,
             o_ref, kbuf, vbuf, wqb, wob, wgb, wub, wdb, xs, ksem, vsem, wsem):
        def kcopy(i, c):
            slot = i % NR
            return pltpu.make_async_copy(k_hbm.at[i % B, i // B, pl.ds(c * CH, CH)],
                                         kbuf.at[slot, pl.ds(c * CH, CH)], ksem.at[slot, c])
        def vcopy(i, c):
            slot = i % NR
            return pltpu.make_async_copy(v_hbm.at[i % B, i // B, pl.ds(c * CH, CH)],
                                         vbuf.at[slot, pl.ds(c * CH, CH)], vsem.at[slot, c])
        def wq_copy(h):
            return pltpu.make_async_copy(wq_hbm.at[:, pl.ds(pl.multiple_of(h * 128, 128), 128)], wqb.at[h % 2], wsem.at[0, h % 2])
        def wo_copy(h):
            return pltpu.make_async_copy(wo_hbm.at[pl.ds(pl.multiple_of(h * 128, 128), 128), :], wob.at[h % 2], wsem.at[1, h % 2])
        def wg_copy(j):
            return pltpu.make_async_copy(wg_hbm.at[:, pl.ds(pl.multiple_of(j * 128, 128), 128)], wgb.at[j % 2], wsem.at[2, j % 2])
        def wu_copy(j):
            return pltpu.make_async_copy(wu_hbm.at[:, pl.ds(pl.multiple_of(j * 128, 128), 128)], wub.at[j % 2], wsem.at[3, j % 2])
        def wd_copy(j):
            return pltpu.make_async_copy(wd_hbm.at[pl.ds(pl.multiple_of(j * 128, 128), 128), :], wdb.at[j % 2], wsem.at[4, j % 2])

        wq_copy(0).start()
        for i in range(NR):
            for c in range(NC):
                kcopy(i, c).start()
            for c in range(NC):
                vcopy(i, c).start()
            if i == 0:
                wo_copy(0).start()
                wg_copy(0).start(); wu_copy(0).start(); wd_copy(0).start()

        xs[...] = jnp.zeros(xs.shape, f32)
        xs[0:B, :] = ax_ref[...].astype(f32)
        xa = xs[0:8, :]
        xb = xa
        xa16 = xa.astype(bf16)
        xb16 = xa16
        row = jax.lax.broadcasted_iota(jnp.int32, (8, 128), 0)

        def head(h, carry):
            acc_a, acc_y = carry
            @pl.when(h + 1 < H)
            def _():
                wq_copy(h + 1).start()
                wo_copy(h + 1).start()
            @pl.when(h + 1 < NF)
            def _():
                wg_copy(h + 1).start(); wu_copy(h + 1).start(); wd_copy(h + 1).start()
            wq_copy(h).wait()
            q = jnp.dot(xa16, wqb[h % 2], preferred_element_type=f32).astype(bf16)
            o_h = jnp.zeros((8, 128), f32)
            for b in range(B):
                i = h * B + b
                slot = i % NR
                ss = []
                for c in range(NC):
                    kcopy(i, c).wait()
                    kk = kbuf[slot, pl.ds(c * CH, CH), :]
                    ss.append(jax.lax.dot_general(q, kk, (((1,), (1,)), ((), ())), preferred_element_type=f32) * scale)
                @pl.when(i + NR < NI)
                def _():
                    for c in range(NC):
                        kcopy(i + NR, c).start()
                m = functools.reduce(jnp.maximum, [jnp.max(s, axis=-1, keepdims=True) for s in ss])
                l = jnp.zeros((8, 1), f32)
                o = jnp.zeros((8, 128), f32)
                for c in range(NC):
                    p = jnp.exp(ss[c] - m)
                    l = l + jnp.sum(p, axis=-1, keepdims=True)
                    vcopy(i, c).wait()
                    o = o + jnp.dot(p.astype(bf16), vbuf[slot, pl.ds(c * CH, CH), :], preferred_element_type=f32)
                @pl.when(i + NR < NI)
                def _():
                    for c in range(NC):
                        vcopy(i + NR, c).start()
                o_h = jnp.where(row == b, o / l, o_h)
            wo_copy(h).wait()
            acc_a = acc_a + jnp.dot(o_h.astype(bf16), wob[h % 2], preferred_element_type=f32)

            def ffn(acc_y):
                wg_copy(h).wait(); wu_copy(h).wait(); wd_copy(h).wait()
                g = jnp.dot(xb16, wgb[h % 2], preferred_element_type=f32)
                u = jnp.dot(xb16, wub[h % 2], preferred_element_type=f32)
                a = (g * jax.nn.sigmoid(g)) * u
                return acc_y + jnp.dot(a.astype(bf16), wdb[h % 2], preferred_element_type=f32)
            acc_y = jax.lax.cond(h < NF, ffn, lambda a: a, acc_y)
            return acc_a, acc_y

        acc_a, acc_y = jax.lax.fori_loop(0, H, head, (jnp.zeros((8, D), f32), jnp.zeros((8, D), f32)))
        gw = gw_ref[...].astype(f32).reshape(1, D)
        wr = wr_ref[...].astype(f32).reshape(1, D)
        gate = jax.nn.sigmoid(jnp.sum(xa * gw, axis=-1, keepdims=True))
        r = jnp.sum(xb * wr, axis=-1, keepdims=True)
        bout = xb + (xb * 0.0 + acc_y * jax.nn.sigmoid(r))
        out = gate * acc_a + (1.0 - gate) * bout
        o_ref[...] = out[0:B, :].astype(o_ref.dtype)

    anyspec = pl.BlockSpec(memory_space=pl.ANY)
    vm = pl.BlockSpec(memory_space=pltpu.VMEM)
    call = pl.pallas_call(
        kern,
        out_shape=jax.ShapeDtypeStruct((B, D), bf16),
        in_specs=[vm, anyspec, anyspec, anyspec, anyspec, vm, anyspec, anyspec, anyspec, vm],
        out_specs=vm,
        scratch_shapes=[
            pltpu.VMEM((NR, Sk, Dh), bf16), pltpu.VMEM((NR, Sk, Dh), bf16),
            pltpu.VMEM((2, D, 128), bf16), pltpu.VMEM((2, 128, D), bf16),
            pltpu.VMEM((2, D, 128), bf16), pltpu.VMEM((2, D, 128), bf16), pltpu.VMEM((2, 128, D), bf16),
            pltpu.VMEM((8, D), f32),
            pltpu.SemaphoreType.DMA((NR, NC)), pltpu.SemaphoreType.DMA((NR, NC)), pltpu.SemaphoreType.DMA((5, 2)),
        ],
        compiler_params=pltpu.CompilerParams(vmem_limit_bytes=vmem_mb * 1024 * 1024),
    )
    def wrapped(ax, k, v, wq, wo, bx, wr, wg, wu, wd, gw):
        return call(ax.reshape(B, D), k, v, wq, wo, wr, wg, wu, wd, gw).reshape(B, 1, D)
    return wrapped


@jax.jit
def pallas_gated_mix__mha_block_cached__moe_arch_mod__decode_kernel(
    A_x, A_k_cache, A_v_cache, A_wq, A_wo, B_x, B_w_r, B_w_gate, B_w_up, B_w_down, gate_w):
    return build()(A_x, A_k_cache, A_v_cache, A_wq, A_wo, B_x, B_w_r, B_w_gate, B_w_up, B_w_down, gate_w)
```

```python
import functools
import jax
import jax.numpy as jnp
import jax.experimental.pallas as pl
import jax.experimental.pallas.tpu as pltpu


def build(CH=1024, PART=64, WPART=64, S=4, vmem_mb=100, nodma=False, nocompute=False):
    B, D, H, Sk, Dh, F = 4, 1024, 32, 8192, 128, 3584
    NC = Sk // CH
    NF = F // 128
    NS = 2 * NC
    assert NS % S == 0
    scale = Dh ** -0.5
    f32, bf16 = jnp.float32, jnp.bfloat16

    def kern(x_hbm, k_hbm, v_hbm, wq_hbm, wo_hbm, wr_hbm, wg_hbm, wu_hbm, wd_hbm, gw_hbm,
             o_ref, ring, wqb, wob, wgb, wub, wdb, xb, wrb, gwb, xs, rsem, wsem, fsem, ssem):

        def start_chunk(src, h, c, slot):
            if nodma: return
            for bb in range(2):
                for r0 in range(0, CH, PART):
                    sz = min(PART, CH - r0)
                    for q in range(2):
                        b = bb + 2 * q
                        pltpu.make_async_copy(src.at[b, h, pl.ds(c * CH + r0, sz)],
                                              ring.at[slot, b, pl.ds(r0, sz)], rsem.at[slot]).start(priority=q)

        def wait_chunk(slot):
            if nodma: return
            pltpu.make_async_copy(ring.at[slot], ring.at[slot], rsem.at[slot]).wait()

        def start_cols(src, dst, j, sem):
            col = pl.ds(pl.multiple_of(j * 128, 128), 128)
            for n, r0 in enumerate(range(0, D // 2, WPART)):
                for q in range(2):
                    rr = pl.ds(r0 + q * (D // 2), WPART)
                    pltpu.make_async_copy(src.at[rr, col], dst.at[rr, :], sem).start(priority=q)

        def start_rows(src, dst, j, sem):
            for r0 in range(0, 64, 16):
                for c0 in range(0, D, 512):
                    for q in range(2):
                        pltpu.make_async_copy(src.at[pl.ds(pl.multiple_of(j * 128 + q * 64 + r0, 16), 16), pl.ds(c0, 512)],
                                              dst.at[pl.ds(q * 64 + r0, 16), pl.ds(c0, 512)], sem).start(priority=q)

        def start_attn_w(h):
            if nodma: return
            start_cols(wq_hbm, wqb.at[h % 2], h, wsem.at[h % 2])
            start_rows(wo_hbm, wob.at[h % 2], h, wsem.at[h % 2])

        def wait_attn_w(h):
            if nodma: return
            pltpu.make_async_copy(wqb.at[h % 2], wqb.at[h % 2], wsem.at[h % 2]).wait()
            pltpu.make_async_copy(wob.at[h % 2], wob.at[h % 2], wsem.at[h % 2]).wait()

        def start_ffn_w(j):
            if nodma: return
            start_cols(wg_hbm, wgb.at[j % 2], j, fsem.at[j % 2])
            start_cols(wu_hbm, wub.at[j % 2], j, fsem.at[j % 2])
            start_rows(wd_hbm, wdb.at[j % 2], j, fsem.at[j % 2])

        def wait_ffn_w(j):
            if nodma: return
            for buf in (wgb, wub, wdb):
                pltpu.make_async_copy(buf.at[j % 2], buf.at[j % 2], fsem.at[j % 2]).wait()

        def start_step(h, t):
            slot = t % S
            if t >= NS:
                h, t = h + 1, t - NS
            if t < NC:
                start_chunk(k_hbm, h, t, slot)
            else:
                start_chunk(v_hbm, h, t - NC, slot)

        def refill(h, t):
            if t + S < NS:
                start_step(h, t + S)
            else:
                @pl.when(h + 1 < H)
                def _():
                    start_step(h, t + S)

        small = [pltpu.make_async_copy(x_hbm, xb, ssem.at[0]),
                 pltpu.make_async_copy(wr_hbm, wrb, ssem.at[1]),
                 pltpu.make_async_copy(gw_hbm, gwb, ssem.at[2])]
        start_attn_w(0)
        for cp in small:
            cp.start()
        for t in range(S):
            start_step(0, t)
        start_ffn_w(0)
        for cp in small:
            cp.wait()

        xs[...] = jnp.zeros(xs.shape, f32)
        xs[0:B, :] = xb[...].astype(f32)
        xf = xs[...]
        x16 = xf.astype(bf16)
        row_s = jax.lax.broadcasted_iota(jnp.int32, (8, CH), 0)
        row_o = jax.lax.broadcasted_iota(jnp.int32, (8, Dh), 0)

        def merge(row, parts):
            r = parts[B - 1]
            for b in range(B - 2, -1, -1):
                r = jnp.where(row == b, parts[b], r)
            return r

        def head(h, carry):
            acc_a, acc_y = carry
            wait_attn_w(h)
            q = jnp.dot(x16, wqb[h % 2], preferred_element_type=f32).astype(bf16)
            ss = []
            for c in range(NC):
                wait_chunk(c % S)
                if not nocompute:
                    parts = [jax.lax.dot_general(q, ring[c % S, b], (((1,), (1,)), ((), ())),
                                                 preferred_element_type=f32) for b in range(B)]
                    ss.append(merge(row_s, parts) * scale)
                refill(h, c)
                if c == 0:
                    @pl.when(h + 1 < H)
                    def _():
                        start_attn_w(h + 1)
                if c == NC // 2:
                    @pl.when(h + 1 < NF)
                    def _():
                        start_ffn_w(h + 1)
            l = jnp.zeros((8, 1), f32)
            o = jnp.zeros((8, Dh), f32)
            if not nocompute:
                m = jnp.max(functools.reduce(jnp.maximum, ss), axis=-1, keepdims=True)
            for c in range(NC):
                if not nocompute:
                    p = jnp.exp(ss[c] - m)
                    l = l + jnp.sum(p, axis=-1, keepdims=True)
                    p16 = p.astype(bf16)
                wait_chunk((NC + c) % S)
                if not nocompute:
                    parts = [jnp.dot(p16, ring[(NC + c) % S, b], preferred_element_type=f32) for b in range(B)]
                    o = o + merge(row_o, parts)
                refill(h, NC + c)
            acc_a = acc_a + jnp.dot((o / l).astype(bf16), wob[h % 2], preferred_element_type=f32)

            def ffn(acc):
                wait_ffn_w(h)
                g = jnp.dot(x16, wgb[h % 2], preferred_element_type=f32)
                u = jnp.dot(x16, wub[h % 2], preferred_element_type=f32)
                a = (g * jax.nn.sigmoid(g)) * u
                return acc + jnp.dot(a.astype(bf16), wdb[h % 2], preferred_element_type=f32)
            acc_y = jax.lax.cond(h < NF, ffn, lambda a: a, acc_y)
            return acc_a, acc_y

        acc_a, acc_y = jax.lax.fori_loop(0, H, head, (jnp.zeros((8, D), f32), jnp.zeros((8, D), f32)))
        gw = gwb[...].astype(f32).reshape(1, D)
        wr = wrb[...].astype(f32).reshape(1, D)
        gate = jax.nn.sigmoid(jnp.sum(xf * gw, axis=-1, keepdims=True))
        r = jnp.sum(xf * wr, axis=-1, keepdims=True)
        bout = xf + (xf * 0.0 + acc_y * jax.nn.sigmoid(r))
        out = gate * acc_a + (1.0 - gate) * bout
        o_ref[...] = out[0:B, :].astype(o_ref.dtype)

    anyspec = pl.BlockSpec(memory_space=pl.ANY)
    call = pl.pallas_call(
        kern,
        out_shape=jax.ShapeDtypeStruct((B, D), bf16),
        in_specs=[anyspec] * 10,
        out_specs=pl.BlockSpec(memory_space=pltpu.VMEM),
        scratch_shapes=[
            pltpu.VMEM((S, B, CH, Dh), bf16),
            pltpu.VMEM((2, D, 128), bf16), pltpu.VMEM((2, 128, D), bf16),
            pltpu.VMEM((2, D, 128), bf16), pltpu.VMEM((2, D, 128), bf16), pltpu.VMEM((2, 128, D), bf16),
            pltpu.VMEM((B, D), bf16), pltpu.VMEM((D,), bf16), pltpu.VMEM((D,), bf16),
            pltpu.VMEM((8, D), f32),
            pltpu.SemaphoreType.DMA((S,)), pltpu.SemaphoreType.DMA((2,)), pltpu.SemaphoreType.DMA((2,)),
            pltpu.SemaphoreType.DMA((3,)),
        ],
        compiler_params=pltpu.CompilerParams(vmem_limit_bytes=vmem_mb * 1024 * 1024),
    )
    def wrapped(ax, k, v, wq, wo, bx, wr, wg, wu, wd, gw):
        return call(ax.reshape(B, D), k, v, wq, wo, wr, wg, wu, wd, gw).reshape(B, 1, D)
    return wrapped


@jax.jit
def pallas_gated_mix__mha_block_cached__moe_arch_mod__decode_kernel(
    A_x, A_k_cache, A_v_cache, A_wq, A_wo, B_x, B_w_r, B_w_gate, B_w_up, B_w_down, gate_w):
    return build(PART=128, S=8, CH=512)(A_x, A_k_cache, A_v_cache, A_wq, A_wo, B_x, B_w_r, B_w_gate, B_w_up, B_w_down, gate_w)
```

```python
import functools
import jax
import jax.numpy as jnp
import jax.experimental.pallas as pl
import jax.experimental.pallas.tpu as pltpu


def build(CH=1024, PART=64, WPART=64, S=4, QM=0, G=1, ROT=(0,0,0,0), vmem_mb=100, nodma=False, nocompute=False, now=False, nof=False):
    B, D, H, Sk, Dh, F = 4, 1024, 32, 8192, 128, 3584
    NC = Sk // CH
    NF = F // 128
    NS = 2 * NC
    assert NS % S == 0
    scale = Dh ** -0.5
    f32, bf16 = jnp.float32, jnp.bfloat16

    def kern(x_hbm, k_hbm, v_hbm, wq_hbm, wo_hbm, wr_hbm, wg_hbm, wu_hbm, wd_hbm, gw_hbm,
             o_ref, ring, wqb, wob, wgb, wub, wdb, xb, wrb, gwb, xs, rsem, wsem, fsem, ssem):

        def start_chunk(src, h, c, slot):
            if nodma: return
            def go(b, r0, q):
                sz = min(PART, CH - r0)
                pltpu.make_async_copy(src.at[b, h, pl.ds(((c + ROT[b]) % NC) * CH + r0, sz)],
                                      ring.at[slot, b, pl.ds(r0, sz)], rsem.at[slot]).start(priority=q)
            if QM >= 10:
                R = CH // G
                def go2(b, g, r0, q):
                    sz = min(PART, R - r0)
                    pltpu.make_async_copy(src.at[b, h, pl.ds(g * (Sk // G) + c * R + r0, sz)],
                                          ring.at[slot, b, pl.ds(g * R + r0, sz)], rsem.at[slot]).start(priority=q)
                if QM == 13:
                    assert sum(PART) == R
                    r0 = 0
                    for sz in PART:
                        for g in range(G):
                            for bb in range(2):
                                for q in range(2):
                                    b = bb + 2 * q
                                    pltpu.make_async_copy(src.at[b, h, pl.ds(g * (Sk // G) + c * R + r0, sz)],
                                          ring.at[slot, b, pl.ds(g * R + r0, sz)], rsem.at[slot]).start(priority=q)
                        r0 += sz
                elif QM == 10:
                    for g in range(G):
                        for bb in range(2):
                            for r0 in range(0, R, PART):
                                go2(bb, g, r0, 0); go2(bb + 2, g, r0, 1)
                elif QM == 11:
                    for bb in range(2):
                        for g in range(G):
                            for r0 in range(0, R, PART):
                                go2(bb, g, r0, 0); go2(bb + 2, g, r0, 1)
                elif QM == 12:
                    for g in range(G):
                        for bb in range(2):
                            for r0 in range(0, R, PART):
                                go2(bb, g, r0, 0); go2(bb + 2, (g + G // 2) % G, r0, 1)
            elif QM == 0:
                for bb in range(2):
                    for r0 in range(0, CH, PART):
                        go(bb, r0, 0); go(bb + 2, r0, 1)
            elif QM == 1:
                for bb in range(2):
                    for r0 in range(0, CH, PART):
                        go(2 * bb, r0, 0); go(2 * bb + 1, r0, 1)
            elif QM == 2:
                for r0 in range(0, CH, PART):
                    for b in range(B):
                        go(b, r0, b % 2)
            elif QM == 3:
                for b in range(B):
                    for r0 in range(0, CH // 2, PART):
                        go(b, r0, 0); go(b, r0 + CH // 2, 1)
            elif QM == 4:
                for bb in range(2):
                    for r0 in range(0, CH, PART):
                        go(bb, r0, 0); go(3 - bb, r0, 1)
            elif QM == 5:
                for b in range(B):
                    for n, r0 in enumerate(range(0, CH, PART)):
                        go(b, r0, n % 2)

        def wait_chunk(slot):
            if nodma: return
            pltpu.make_async_copy(ring.at[slot], ring.at[slot], rsem.at[slot]).wait()

        def start_cols(src, dst, j, sem):
            col = pl.ds(pl.multiple_of(j * 128, 128), 128)
            for n, r0 in enumerate(range(0, D // 2, WPART)):
                for q in range(2):
                    rr = pl.ds(r0 + q * (D // 2), WPART)
                    pltpu.make_async_copy(src.at[rr, col], dst.at[rr, :], sem).start(priority=q)

        def start_rows(src, dst, j, sem):
            for r0 in range(0, 64, 16):
                for c0 in range(0, D, 512):
                    for q in range(2):
                        pltpu.make_async_copy(src.at[pl.ds(pl.multiple_of(j * 128 + q * 64 + r0, 16), 16), pl.ds(c0, 512)],
                                              dst.at[pl.ds(q * 64 + r0, 16), pl.ds(c0, 512)], sem).start(priority=q)

        def start_attn_w(h):
            if nodma or now: return
            start_cols(wq_hbm, wqb.at[h % 2], h, wsem.at[h % 2])
            start_rows(wo_hbm, wob.at[h % 2], h, wsem.at[h % 2])

        def wait_attn_w(h):
            if nodma or now: return
            pltpu.make_async_copy(wqb.at[h % 2], wqb.at[h % 2], wsem.at[h % 2]).wait()
            pltpu.make_async_copy(wob.at[h % 2], wob.at[h % 2], wsem.at[h % 2]).wait()

        def start_ffn_w(j):
            if nodma or nof: return
            start_cols(wg_hbm, wgb.at[j % 2], j, fsem.at[j % 2])
            start_cols(wu_hbm, wub.at[j % 2], j, fsem.at[j % 2])
            start_rows(wd_hbm, wdb.at[j % 2], j, fsem.at[j % 2])

        def wait_ffn_w(j):
            if nodma or nof: return
            for buf in (wgb, wub, wdb):
                pltpu.make_async_copy(buf.at[j % 2], buf.at[j % 2], fsem.at[j % 2]).wait()

        def start_step(h, t):
            slot = t % S
            if t >= NS:
                h, t = h + 1, t - NS
            if t < NC:
                start_chunk(k_hbm, h, t, slot)
            else:
                start_chunk(v_hbm, h, t - NC, slot)

        def refill(h, t):
            if t + S < NS:
                start_step(h, t + S)
            else:
                @pl.when(h + 1 < H)
                def _():
                    start_step(h, t + S)

        small = [pltpu.make_async_copy(x_hbm, xb, ssem.at[0]),
                 pltpu.make_async_copy(wr_hbm, wrb, ssem.at[1]),
                 pltpu.make_async_copy(gw_hbm, gwb, ssem.at[2])]
        start_attn_w(0)
        for cp in small:
            cp.start()
        for t in range(S):
            start_step(0, t)
        start_ffn_w(0)
        for cp in small:
            cp.wait()

        xs[...] = jnp.zeros(xs.shape, f32)
        xs[0:B, :] = xb[...].astype(f32)
        xf = xs[...]
        x16 = xf.astype(bf16)
        row_s = jax.lax.broadcasted_iota(jnp.int32, (8, CH), 0)
        row_o = jax.lax.broadcasted_iota(jnp.int32, (8, Dh), 0)

        def merge(row, parts):
            r = parts[B - 1]
            for b in range(B - 2, -1, -1):
                r = jnp.where(row == b, parts[b], r)
            return r

        def head(h, carry):
            acc_a, acc_y = carry
            wait_attn_w(h)
            q = jnp.dot(x16, wqb[h % 2], preferred_element_type=f32).astype(bf16)
            ss = []
            for c in range(NC):
                wait_chunk(c % S)
                if not nocompute:
                    parts = [jax.lax.dot_general(q, ring[c % S, b], (((1,), (1,)), ((), ())),
                                                 preferred_element_type=f32) for b in range(B)]
                    ss.append(merge(row_s, parts) * scale)
                refill(h, c)
                if c == 0:
                    @pl.when(h + 1 < H)
                    def _():
                        start_attn_w(h + 1)
                if c == NC // 2:
                    @pl.when(h + 1 < NF)
                    def _():
                        start_ffn_w(h + 1)
            l = jnp.zeros((8, 1), f32)
            o = jnp.zeros((8, Dh), f32)
            if not nocompute:
                m = jnp.max(functools.reduce(jnp.maximum, ss), axis=-1, keepdims=True)
            for c in range(NC):
                if not nocompute:
                    p = jnp.exp(ss[c] - m)
                    l = l + jnp.sum(p, axis=-1, keepdims=True)
                    p16 = p.astype(bf16)
                wait_chunk((NC + c) % S)
                if not nocompute:
                    parts = [jnp.dot(p16, ring[(NC + c) % S, b], preferred_element_type=f32) for b in range(B)]
                    o = o + merge(row_o, parts)
                refill(h, NC + c)
            acc_a = acc_a + jnp.dot((o / l).astype(bf16), wob[h % 2], preferred_element_type=f32)

            def ffn(acc):
                wait_ffn_w(h)
                g = jnp.dot(x16, wgb[h % 2], preferred_element_type=f32)
                u = jnp.dot(x16, wub[h % 2], preferred_element_type=f32)
                a = (g * jax.nn.sigmoid(g)) * u
                return acc + jnp.dot(a.astype(bf16), wdb[h % 2], preferred_element_type=f32)
            acc_y = jax.lax.cond(h < NF, ffn, lambda a: a, acc_y)
            return acc_a, acc_y

        acc_a, acc_y = jax.lax.fori_loop(0, H, head, (jnp.zeros((8, D), f32), jnp.zeros((8, D), f32)))
        gw = gwb[...].astype(f32).reshape(1, D)
        wr = wrb[...].astype(f32).reshape(1, D)
        gate = jax.nn.sigmoid(jnp.sum(xf * gw, axis=-1, keepdims=True))
        r = jnp.sum(xf * wr, axis=-1, keepdims=True)
        bout = xf + (xf * 0.0 + acc_y * jax.nn.sigmoid(r))
        out = gate * acc_a + (1.0 - gate) * bout
        o_ref[...] = out[0:B, :].astype(o_ref.dtype)

    anyspec = pl.BlockSpec(memory_space=pl.ANY)
    call = pl.pallas_call(
        kern,
        out_shape=jax.ShapeDtypeStruct((B, D), bf16),
        in_specs=[anyspec] * 10,
        out_specs=pl.BlockSpec(memory_space=pltpu.VMEM),
        scratch_shapes=[
            pltpu.VMEM((S, B, CH, Dh), bf16),
            pltpu.VMEM((2, D, 128), bf16), pltpu.VMEM((2, 128, D), bf16),
            pltpu.VMEM((2, D, 128), bf16), pltpu.VMEM((2, D, 128), bf16), pltpu.VMEM((2, 128, D), bf16),
            pltpu.VMEM((B, D), bf16), pltpu.VMEM((D,), bf16), pltpu.VMEM((D,), bf16),
            pltpu.VMEM((8, D), f32),
            pltpu.SemaphoreType.DMA((S,)), pltpu.SemaphoreType.DMA((2,)), pltpu.SemaphoreType.DMA((2,)),
            pltpu.SemaphoreType.DMA((3,)),
        ],
        compiler_params=pltpu.CompilerParams(vmem_limit_bytes=vmem_mb * 1024 * 1024),
    )
    def wrapped(ax, k, v, wq, wo, bx, wr, wg, wu, wd, gw):
        return call(ax.reshape(B, D), k, v, wq, wo, wr, wg, wu, wd, gw).reshape(B, 1, D)
    return wrapped


@jax.jit
def pallas_gated_mix__mha_block_cached__moe_arch_mod__decode_kernel(
    A_x, A_k_cache, A_v_cache, A_wq, A_wo, B_x, B_w_r, B_w_gate, B_w_up, B_w_down, gate_w):
    return build(PART=(96,96,64),S=4,CH=1024,G=4,QM=13,WPART=128)(A_x, A_k_cache, A_v_cache, A_wq, A_wo, B_x, B_w_r, B_w_gate, B_w_up, B_w_down, gate_w)
```

```python
import functools
import jax
import jax.numpy as jnp
import jax.experimental.pallas as pl
import jax.experimental.pallas.tpu as pltpu


def build(PART=(96, 96, 64), G=4, S=4, NG=2, WB=16, WC=512, TA=0, TF=4, nobc=True, HH=32, vmem_mb=100):
    B, D, H, Sk, Dh, F = 4, 1024, 32, 8192, 128, 3584
    R = sum(PART)
    CH = G * R
    NC = Sk // CH
    NS = 2 * NC
    GW = 128 * NG
    NF = F // GW
    RW = D // NG
    assert Sk % CH == 0 and S <= NC
    scale = Dh ** -0.5
    f32, bf16 = jnp.float32, jnp.bfloat16

    def kern(x_hbm, k_hbm, v_hbm, wq_hbm, wo_hbm, wr_hbm, wg_hbm, wu_hbm, wd_hbm, gw_hbm,
             o_ref, ring, wqb, wob, wgb, wub, wdb, xb, wrb, gwb, xs, q3, sbuf, ybuf, pre,
             rsem, wsem, osem, fsem, ssem):

        def wait_all(buf, sem):
            pltpu.make_async_copy(buf, buf, sem).wait()

        def col_pieces(src, dst, h, sem):
            j = h // NG
            col = pl.ds(pl.multiple_of(j * GW, GW), GW)
            wr = WB * 1024 // (GW * 2)
            out = []
            for r0 in range(0, RW, wr):
                rr = pl.ds(pl.multiple_of((h % NG) * RW + r0, 16), min(wr, RW - r0))
                out.append(pltpu.make_async_copy(src.at[rr, col], dst.at[j % 2, rr, :], sem))
            return out

        def row_pieces(src, dst, h, sem):
            out = []
            for c0 in range(0, D, WC):
                cs = pl.ds(c0, min(WC, D - c0))
                for r0 in (0, 64, 16, 80, 32, 96, 48, 112):
                    out.append(pltpu.make_async_copy(
                        src.at[pl.ds(pl.multiple_of(h * 128 + r0, 16), 16), cs], dst.at[pl.ds(r0, 16), cs], sem))
            return out

        def start_all(pieces):
            for n, p in enumerate(pieces):
                p.start(priority=n % 2)

        def start_wq(h):
            start_all(col_pieces(wq_hbm, wqb, h, wsem.at[(h // NG) % 2]))

        def start_ffn(h):
            sl = (h // NG) % 2
            start_all(col_pieces(wg_hbm, wgb, h, fsem.at[sl]) + col_pieces(wu_hbm, wub, h, fsem.at[sl])
                      + row_pieces(wd_hbm, wdb.at[sl, h % NG], h, fsem.at[sl]))

        def start_chunk(src, h, c, slot):
            r0 = 0
            for sz in PART:
                for g in range(G):
                    for bb in range(2):
                        for q in range(2):
                            b = bb + 2 * q
                            pltpu.make_async_copy(
                                src.at[b, h, pl.ds(pl.multiple_of(g * (Sk // G) + c * R + r0, 16), sz)],
                                ring.at[slot, b, pl.ds(g * R + r0, sz)], rsem.at[slot]).start(priority=q)
                r0 += sz

        def start_step(t):
            h, r, slot = t // NS, t % NS, t % S
            @pl.when(r < NC)
            def _():
                start_chunk(k_hbm, h, r, slot)
            @pl.when(r >= NC)
            def _():
                start_chunk(v_hbm, h, r - NC, slot)

        def refill(h, r):
            t = h * NS + r + S
            @pl.when(t < HH * NS)
            def _():
                start_step(t)

        small = [pltpu.make_async_copy(x_hbm, xb, ssem.at[0]),
                 pltpu.make_async_copy(wr_hbm, wrb, ssem.at[1]),
                 pltpu.make_async_copy(gw_hbm, gwb, ssem.at[2])]
        for cp in small:
            cp.start()
        pl.loop(0, NG)(start_wq)
        pl.loop(0, S)(lambda t: start_chunk(k_hbm, 0, t, t))
        pl.loop(0, NG)(start_ffn)
        for cp in small:
            cp.wait()

        xs[...] = jnp.zeros(xs.shape, f32)
        xs[0:B, :] = xb[...].astype(f32)
        ybuf[...] = jnp.zeros(ybuf.shape, f32)
        row_s = jax.lax.broadcasted_iota(jnp.int32, (8, CH), 0)
        row_o = jax.lax.broadcasted_iota(jnp.int32, (8, Dh), 0)

        def merge(row, parts):
            r = parts[B - 1]
            for b in range(B - 2, -1, -1):
                r = jnp.where(row == b, parts[b], r)
            return r

        def fold(a, op):
            return functools.reduce(op, [a[:, i:i + 128] for i in range(0, CH, 128)])

        def head(h, acc_a):
            sl = (h // NG) % 2
            @pl.when(h % NG == 0)
            def _():
                wait_all(wqb.at[sl], wsem.at[sl])
                qg = jnp.dot(xs[...].astype(bf16), wqb[sl], preferred_element_type=f32).astype(bf16)
                for n in range(NG):
                    q3[n] = qg[:, n * Dh:(n + 1) * Dh]
            q = q3[h % NG]

            def kstep(c, mv):
                slot = (h * NS + c) % S
                wait_all(ring.at[slot], rsem.at[slot])
                parts = [jax.lax.dot_general(q, ring[slot, b], (((1,), (1,)), ((), ())),
                                             preferred_element_type=f32) for b in range(B)]
                s = merge(row_s, parts) * scale
                sbuf[c] = s
                refill(h, c)
                @pl.when(jnp.logical_and(c == TA, h + NG < HH))
                def _():
                    start_wq(h + NG)
                @pl.when(jnp.logical_and(c == TF, h + NG < min(HH, NF * NG)))
                def _():
                    start_ffn(h + NG)
                return jnp.maximum(mv, fold(s, jnp.maximum))
            mv = jax.lax.fori_loop(0, NC, kstep, jnp.full((8, 128), -jnp.inf, f32))
            m = jnp.max(mv, axis=-1, keepdims=True)

            @pl.when(jnp.logical_and(h % NG == NG - 1, h < min(HH, NF * NG)))
            def _():
                for buf in (wgb, wub, wdb):
                    wait_all(buf.at[sl], fsem.at[sl])
                x16 = xs[...].astype(bf16)
                g = jnp.dot(x16, wgb[sl], preferred_element_type=f32)
                u = jnp.dot(x16, wub[sl], preferred_element_type=f32)
                a = (g * jax.nn.sigmoid(g)) * u
                ybuf[...] += jnp.dot(a.astype(bf16), wdb[sl].reshape(GW, D), preferred_element_type=f32)

            @pl.when(h == HH - 1)
            def _():
                xf = xs[...]
                gw = gwb[...].astype(f32).reshape(1, D)
                wr = wrb[...].astype(f32).reshape(1, D)
                gate = jax.nn.sigmoid(jnp.sum(xf * gw, axis=-1, keepdims=True))
                r = jnp.sum(xf * wr, axis=-1, keepdims=True)
                bout = xf + (xf * 0.0 + ybuf[...] * jax.nn.sigmoid(r))
                pre[0] = jnp.broadcast_to(gate, (8, D))
                pre[1] = (1.0 - gate) * bout

            def vstep(c, carry):
                lv, o = carry
                slot = (h * NS + NC + c) % S
                p = jnp.exp(sbuf[c] - m)
                lv = lv + fold(p, jnp.add)
                p16 = p.astype(bf16)
                wait_all(ring.at[slot], rsem.at[slot])
                parts = [jnp.dot(p16, ring[slot, b], preferred_element_type=f32) for b in range(B)]
                o = o + merge(row_o, parts)
                refill(h, NC + c)
                @pl.when(c == NC - S - 1 if S < NC else False)
                def _():
                    start_all(row_pieces(wo_hbm, wob, h, osem))
                return lv, o
            lv, o = jax.lax.fori_loop(0, NC, vstep, (jnp.zeros((8, 128), f32), jnp.zeros((8, Dh), f32)))
            o = o / jnp.sum(lv, axis=-1, keepdims=True)
            wait_all(wob, osem)
            return acc_a + jnp.dot(o.astype(bf16), wob[...], preferred_element_type=f32)

        acc_a = jax.lax.fori_loop(0, HH, head, jnp.zeros((8, D), f32))
        out = pre[0] * acc_a + pre[1]
        o_ref[...] = out[0:B, :].astype(o_ref.dtype)

    assert S < NC
    anyspec = pl.BlockSpec(memory_space=pl.ANY)
    DMA = pltpu.SemaphoreType.DMA
    call = pl.pallas_call(
        kern,
        out_shape=jax.ShapeDtypeStruct((B, D), bf16),
        in_specs=[anyspec] * 10,
        out_specs=pl.BlockSpec(memory_space=pltpu.VMEM),
        scratch_shapes=[
            pltpu.VMEM((S, B, CH, Dh), bf16),
            pltpu.VMEM((2, D, GW), bf16), pltpu.VMEM((128, D), bf16),
            pltpu.VMEM((2, D, GW), bf16), pltpu.VMEM((2, D, GW), bf16), pltpu.VMEM((2, NG, 128, D), bf16),
            pltpu.VMEM((B, D), bf16), pltpu.VMEM((D,), bf16), pltpu.VMEM((D,), bf16),
            pltpu.VMEM((8, D), f32), pltpu.VMEM((NG, 8, Dh), bf16),
            pltpu.VMEM((NC, 8, CH), f32), pltpu.VMEM((8, D), f32), pltpu.VMEM((2, 8, D), f32),
            DMA((S,)), DMA((2,)), DMA(()), DMA((2,)), DMA((3,)),
        ],
        compiler_params=pltpu.CompilerParams(vmem_limit_bytes=vmem_mb * 1024 * 1024, disable_bounds_checks=nobc),
    )
    def wrapped(ax, k, v, wq, wo, bx, wr, wg, wu, wd, gw):
        return call(ax.reshape(B, D), k, v, wq, wo, wr, wg, wu, wd, gw).reshape(B, 1, D)
    return wrapped


@jax.jit
def pallas_gated_mix__mha_block_cached__moe_arch_mod__decode_kernel(
    A_x, A_k_cache, A_v_cache, A_wq, A_wo, B_x, B_w_r, B_w_gate, B_w_up, B_w_down, gate_w):
    return build()(A_x, A_k_cache, A_v_cache, A_wq, A_wo, B_x, B_w_r, B_w_gate, B_w_up, B_w_down, gate_w)
```

```python
import functools
import jax
import jax.numpy as jnp
import jax.experimental.pallas as pl
import jax.experimental.pallas.tpu as pltpu


def build(PART=(96, 96, 64), G=4, S=4, QW=(1280, 1280, 1536), FW=(1280, 1280, 1024), RP=(8, 8, 8, 8), TW=0,
          nobc=True, vmem_mb=100):
    B, D, H, Sk, Dh, F = 4, 1024, 32, 8192, 128, 3584
    R = sum(PART)
    CH = G * R
    NC = Sk // CH
    NS = 2 * NC
    FS = 512
    NF = F // FS
    HG = H // NC
    assert Sk % CH == 0 and S <= NC and TW < NC and H % NC == 0
    assert sum(QW) == H * Dh and sum(FW) == F and sum(RP) == 32
    T_WD, T_WO, T_END = 16, 16 + NF, 16 + NF + 8
    assert T_END < H
    scale = Dh ** -0.5
    f32, bf16 = jnp.float32, jnp.bfloat16

    def kern(x_hbm, k_hbm, v_hbm, wq_hbm, wo_hbm, wr_hbm, wg_hbm, wu_hbm, wd_hbm, gw_hbm,
             o_ref, ring, wqb, wob, wgb, wub, wdb, xb, wrb, gwb, xs, o3, sbuf, ybuf, abuf,
             rsem, wsem, ssem):

        def wait_all(buf, sem):
            pltpu.make_async_copy(buf, buf, sem).wait()

        def copy(src, dst, rows, cols, sem, q):
            pltpu.make_async_copy(src.at[rows, cols], dst.at[rows, cols], sem).start(priority=q)

        def start_wq(c):
            c0 = 0
            for sz in QW:
                for st in range(8):
                    for q in range(2):
                        rows = pl.ds(pl.multiple_of((st + 8 * q) * 64 + c * 8, 8), 8)
                        copy(wq_hbm, wqb, rows, pl.ds(c0, sz), wsem.at[0], q)
                c0 += sz

        def start_gu(c):
            c0 = 0
            for sz in FW:
                for st in range(8):
                    rows = pl.ds(pl.multiple_of(st * 128 + c * 8, 8), 8)
                    copy(wg_hbm, wgb, rows, pl.ds(c0, sz), wsem.at[1], 0)
                    copy(wu_hbm, wub, rows, pl.ds(c0, sz), wsem.at[1], 1)
                c0 += sz

        def start_tall(src, dst, sem, c):
            per = dst.shape[0] // 16
            r0 = 0
            for sz in RP:
                for st in range(8):
                    for q in range(2):
                        rows = pl.ds(pl.multiple_of((st + 8 * q) * per + c * 32 + r0, 8), sz)
                        copy(src, dst, rows, slice(None), sem, q)
                r0 += sz

        def start_weights(h):
            @pl.when(h < T_WD)
            def _():
                start_gu(h)
            @pl.when(jnp.logical_and(h >= T_WD, h < T_WO))
            def _():
                start_tall(wd_hbm, wdb, wsem.at[2], h - T_WD)
            @pl.when(jnp.logical_and(h >= T_WO, h < T_END))
            def _():
                start_tall(wo_hbm, wob, wsem.at[3], h - T_WO)

        def start_chunk(src, h, c, slot):
            r0 = 0
            for sz in PART:
                for g in range(G):
                    for bb in range(2):
                        for q in range(2):
                            b = bb + 2 * q
                            pltpu.make_async_copy(
                                src.at[b, h, pl.ds(pl.multiple_of(g * (Sk // G) + c * R + r0, 8), sz)],
                                ring.at[slot, b, pl.ds(g * R + r0, sz)], rsem.at[slot]).start(priority=q)
                r0 += sz

        def refill(h, r):
            t = h * NS + r + S
            hh, rr, slot = t // NS, t % NS, t % S
            @pl.when(jnp.logical_and(hh < H, rr < NC))
            def _():
                start_chunk(k_hbm, hh, rr, slot)
            @pl.when(jnp.logical_and(hh < H, rr >= NC))
            def _():
                start_chunk(v_hbm, hh, rr - NC, slot)

        small = [pltpu.make_async_copy(x_hbm, xb, ssem.at[0]),
                 pltpu.make_async_copy(wr_hbm, wrb, ssem.at[1]),
                 pltpu.make_async_copy(gw_hbm, gwb, ssem.at[2])]
        for cp in small:
            cp.start()
        pl.loop(0, 8)(start_wq)
        pl.loop(0, S)(lambda t: start_chunk(k_hbm, 0, t, t))
        for cp in small:
            cp.wait()

        xs[...] = jnp.zeros(xs.shape, f32)
        xs[0:B, :] = xb[...].astype(f32)
        ybuf[...] = jnp.zeros(ybuf.shape, f32)
        abuf[...] = jnp.zeros(abuf.shape, f32)
        row_s = jax.lax.broadcasted_iota(jnp.int32, (8, CH), 0)
        row_o = jax.lax.broadcasted_iota(jnp.int32, (8, Dh), 0)
        wait_all(wqb, wsem.at[0])

        def merge(row, parts):
            r = parts[B - 1]
            for b in range(B - 2, -1, -1):
                r = jnp.where(row == b, parts[b], r)
            return r

        def fold(a, op):
            return functools.reduce(op, [a[:, i:i + 128] for i in range(0, CH, 128)])

        def project(hh):
            rows = pl.ds(pl.multiple_of(hh * Dh, Dh), Dh)
            abuf[...] += jnp.dot(o3[hh], wob[rows, :], preferred_element_type=f32)

        def head(h, _):
            q = jnp.dot(xs[...].astype(bf16), wqb[:, pl.ds(pl.multiple_of(h * Dh, Dh), Dh)],
                        preferred_element_type=f32).astype(bf16)

            def kstep(c, mv):
                slot = (h * NS + c) % S
                wait_all(ring.at[slot], rsem.at[slot])
                parts = [jax.lax.dot_general(q, ring[slot, b], (((1,), (1,)), ((), ())),
                                             preferred_element_type=f32) for b in range(B)]
                s = merge(row_s, parts) * scale
                sbuf[c] = s
                refill(h, c)
                @pl.when(c == TW)
                def _():
                    start_weights(h)
                @pl.when(h == H - 1)
                def _():
                    @pl.when(c == 0)
                    def _():
                        wait_all(wob, wsem.at[3])
                    pl.loop(c * HG, jnp.minimum((c + 1) * HG, H - 1))(project)
                return jnp.maximum(mv, fold(s, jnp.maximum))
            mv = jax.lax.fori_loop(0, NC, kstep, jnp.full((8, 128), -jnp.inf, f32))
            m = jnp.max(mv, axis=-1, keepdims=True)

            @pl.when(h == T_WO)
            def _():
                wait_all(wgb, wsem.at[1])
                wait_all(wub, wsem.at[1])
                wait_all(wdb, wsem.at[2])

            @pl.when(jnp.logical_and(h >= T_WO, h < T_WO + NF))
            def _():
                sl = pl.ds(pl.multiple_of((h - T_WO) * FS, FS), FS)
                x16 = xs[...].astype(bf16)
                g = jnp.dot(x16, wgb[:, sl], preferred_element_type=f32)
                u = jnp.dot(x16, wub[:, sl], preferred_element_type=f32)
                a = (g * jax.nn.sigmoid(g)) * u
                ybuf[...] += jnp.dot(a.astype(bf16), wdb[sl, :], preferred_element_type=f32)

            @pl.when(h == H - 2)
            def _():
                xf = xs[...]
                wr = wrb[...].astype(f32).reshape(1, D)
                r = jnp.sum(xf * wr, axis=-1, keepdims=True)
                ybuf[...] = xf + (xf * 0.0 + ybuf[...] * jax.nn.sigmoid(r))

            def vstep(c, carry):
                lv, o = carry
                slot = (h * NS + NC + c) % S
                p = jnp.exp(sbuf[c] - m)
                lv = lv + fold(p, jnp.add)
                p16 = p.astype(bf16)
                wait_all(ring.at[slot], rsem.at[slot])
                parts = [jnp.dot(p16, ring[slot, b], preferred_element_type=f32) for b in range(B)]
                o = o + merge(row_o, parts)
                refill(h, NC + c)
                return lv, o
            lv, o = jax.lax.fori_loop(0, NC, vstep, (jnp.zeros((8, 128), f32), jnp.zeros((8, Dh), f32)))
            o3[h] = (o / jnp.sum(lv, axis=-1, keepdims=True)).astype(bf16)

        gw = gwb[...].astype(f32).reshape(1, D)
        gate = jax.nn.sigmoid(jnp.sum(xs[...] * gw, axis=-1, keepdims=True))
        jax.lax.fori_loop(0, H, head, None)
        project(H - 1)
        out = gate * abuf[...] + (1.0 - gate) * ybuf[...]
        o_ref[...] = out[0:B, :].astype(o_ref.dtype)

    anyspec = pl.BlockSpec(memory_space=pl.ANY)
    DMA = pltpu.SemaphoreType.DMA
    call = pl.pallas_call(
        kern,
        out_shape=jax.ShapeDtypeStruct((B, D), bf16),
        in_specs=[anyspec] * 10,
        out_specs=pl.BlockSpec(memory_space=pltpu.VMEM),
        scratch_shapes=[
            pltpu.VMEM((S, B, CH, Dh), bf16),
            pltpu.VMEM((D, H * Dh), bf16), pltpu.VMEM((H * Dh, D), bf16),
            pltpu.VMEM((D, F), bf16), pltpu.VMEM((D, F), bf16), pltpu.VMEM((F, D), bf16),
            pltpu.VMEM((B, D), bf16), pltpu.VMEM((D,), bf16), pltpu.VMEM((D,), bf16),
            pltpu.VMEM((8, D), f32), pltpu.VMEM((H, 8, Dh), bf16),
            pltpu.VMEM((NC, 8, CH), f32), pltpu.VMEM((8, D), f32), pltpu.VMEM((8, D), f32),
            DMA((S,)), DMA((4,)), DMA((3,)),
        ],
        compiler_params=pltpu.CompilerParams(vmem_limit_bytes=vmem_mb * 1024 * 1024, disable_bounds_checks=nobc),
    )
    def wrapped(ax, k, v, wq, wo, bx, wr, wg, wu, wd, gw):
        return call(ax.reshape(B, D), k, v, wq, wo, wr, wg, wu, wd, gw).reshape(B, 1, D)
    return wrapped


@jax.jit
def pallas_gated_mix__mha_block_cached__moe_arch_mod__decode_kernel(
    A_x, A_k_cache, A_v_cache, A_wq, A_wo, B_x, B_w_r, B_w_gate, B_w_up, B_w_down, gate_w):
    return build()(A_x, A_k_cache, A_v_cache, A_wq, A_wo, B_x, B_w_r, B_w_gate, B_w_up, B_w_down, gate_w)
```

```python
import functools
import jax
import jax.numpy as jnp
import jax.experimental.pallas as pl
import jax.experimental.pallas.tpu as pltpu


def build(PART=(96, 96, 64), G=4, S=4, QW=(1280, 1280, 1536), FW=(1280, 1280, 1024), RP=(8, 8, 8, 8), TW=0, ROT=None, STAG=0, ORD=0, PAIR=0,
          nobc=True, vmem_mb=100):
    B, D, H, Sk, Dh, F = 4, 1024, 32, 8192, 128, 3584
    R = sum(PART)
    CH = G * R
    NC = Sk // CH
    NS = 2 * NC
    FS = 512
    NF = F // FS
    HG = H // NC
    assert Sk % CH == 0 and S <= NC and TW < NC and H % NC == 0
    assert sum(QW) == H * Dh and sum(FW) == F and sum(RP) == 32
    T_WD, T_WO, T_END = 16, 16 + NF, 16 + NF + 8
    assert T_END < H
    scale = Dh ** -0.5
    f32, bf16 = jnp.float32, jnp.bfloat16

    def kern(x_hbm, k_hbm, v_hbm, wq_hbm, wo_hbm, wr_hbm, wg_hbm, wu_hbm, wd_hbm, gw_hbm,
             o_ref, ring, wqb, wob, wgb, wub, wdb, xb, wrb, gwb, xs, o3, sbuf, ybuf, abuf,
             rsem, wsem, ssem):

        def wait_all(buf, sem):
            pltpu.make_async_copy(buf, buf, sem).wait()

        def copy(src, dst, rows, cols, sem, q):
            pltpu.make_async_copy(src.at[rows, cols], dst.at[rows, cols], sem).start(priority=q)

        def start_wq(c):
            c0 = 0
            for sz in QW:
                for st in range(8):
                    for q in range(2):
                        rows = pl.ds(pl.multiple_of((st + 8 * q) * 64 + c * 8, 8), 8)
                        copy(wq_hbm, wqb, rows, pl.ds(c0, sz), wsem.at[0], q)
                c0 += sz

        def start_gu(c):
            c0 = 0
            for sz in FW:
                for st in range(8):
                    rows = pl.ds(pl.multiple_of(st * 128 + c * 8, 8), 8)
                    copy(wg_hbm, wgb, rows, pl.ds(c0, sz), wsem.at[1], 0)
                    copy(wu_hbm, wub, rows, pl.ds(c0, sz), wsem.at[1], 1)
                c0 += sz

        def start_tall(src, dst, sem, c):
            per = dst.shape[0] // 16
            r0 = 0
            for sz in RP:
                for st in range(8):
                    for q in range(2):
                        rows = pl.ds(pl.multiple_of((st + 8 * q) * per + c * 32 + r0, 8), sz)
                        copy(src, dst, rows, slice(None), sem, q)
                r0 += sz

        def start_weights(h):
            @pl.when(h < T_WD)
            def _():
                start_gu(h)
            @pl.when(jnp.logical_and(h >= T_WD, h < T_WO))
            def _():
                start_tall(wd_hbm, wdb, wsem.at[2], h - T_WD)
            @pl.when(jnp.logical_and(h >= T_WO, h < T_END))
            def _():
                start_tall(wo_hbm, wob, wsem.at[3], h - T_WO)

        def start_chunk(src, h, c, slot):
            def go(b, g, n, q):
                sid = b * G + g
                k = (STAG * sid) % len(PART)
                part = PART[k:] + PART[:k]
                r0, sz = sum(part[:n]), part[n]
                cc = c if ROT is None else (c + ROT[sid]) % NC
                pltpu.make_async_copy(
                    src.at[b, h, pl.ds(pl.multiple_of(g * (Sk // G) + cc * R + r0, 8), sz)],
                    ring.at[slot, b, pl.ds(g * R + r0, sz)], rsem.at[slot]).start(priority=q)
            def pair(g, bb):
                if PAIR == 0: return (bb, g), (bb + 2, g)
                if PAIR == 1: return (2 * bb, g), (2 * bb + 1, g)
                if PAIR == 2: return (bb, g), (bb + 2, (g + G // 2) % G)
                if PAIR == 3: return (bb, g), (3 - bb, G - 1 - g)
                if PAIR == 4: return (2 * bb + g % 2, g // 2), (2 * bb + g % 2, g // 2 + G // 2)
                if PAIR == 5: return (bb, g), (bb + 2, (g + 1) % G)
            N = len(PART)
            if ORD == 0: seq = [(n, g, bb) for n in range(N) for g in range(G) for bb in range(2)]
            if ORD == 1: seq = [(n, g, bb) for n in range(N) for bb in range(2) for g in range(G)]
            if ORD == 2: seq = [(n, g, bb) for g in range(G) for n in range(N) for bb in range(2)]
            if ORD == 3: seq = [(n, g, bb) for bb in range(2) for n in range(N) for g in range(G)]
            for n, g, bb in seq:
                s0, s1 = pair(g, bb)
                go(*s0, n, 0)
                go(*s1, n, 1)

        def refill(h, r):
            t = h * NS + r + S
            hh, rr, slot = t // NS, t % NS, t % S
            @pl.when(jnp.logical_and(hh < H, rr < NC))
            def _():
                start_chunk(k_hbm, hh, rr, slot)
            @pl.when(jnp.logical_and(hh < H, rr >= NC))
            def _():
                start_chunk(v_hbm, hh, rr - NC, slot)

        small = [pltpu.make_async_copy(x_hbm, xb, ssem.at[0]),
                 pltpu.make_async_copy(wr_hbm, wrb, ssem.at[1]),
                 pltpu.make_async_copy(gw_hbm, gwb, ssem.at[2])]
        for cp in small:
            cp.start()
        pl.loop(0, 8)(start_wq)
        pl.loop(0, S)(lambda t: start_chunk(k_hbm, 0, t, t))
        for cp in small:
            cp.wait()

        xs[...] = jnp.zeros(xs.shape, f32)
        xs[0:B, :] = xb[...].astype(f32)
        ybuf[...] = jnp.zeros(ybuf.shape, f32)
        abuf[...] = jnp.zeros(abuf.shape, f32)
        row_s = jax.lax.broadcasted_iota(jnp.int32, (8, CH), 0)
        row_o = jax.lax.broadcasted_iota(jnp.int32, (8, Dh), 0)
        wait_all(wqb, wsem.at[0])

        def merge(row, parts):
            r = parts[B - 1]
            for b in range(B - 2, -1, -1):
                r = jnp.where(row == b, parts[b], r)
            return r

        def fold(a, op):
            return functools.reduce(op, [a[:, i:i + 128] for i in range(0, CH, 128)])

        def project(hh):
            rows = pl.ds(pl.multiple_of(hh * Dh, Dh), Dh)
            abuf[...] += jnp.dot(o3[hh], wob[rows, :], preferred_element_type=f32)

        def head(h, _):
            q = jnp.dot(xs[...].astype(bf16), wqb[:, pl.ds(pl.multiple_of(h * Dh, Dh), Dh)],
                        preferred_element_type=f32).astype(bf16)

            def kstep(c, mv):
                slot = (h * NS + c) % S
                wait_all(ring.at[slot], rsem.at[slot])
                parts = [jax.lax.dot_general(q, ring[slot, b], (((1,), (1,)), ((), ())),
                                             preferred_element_type=f32) for b in range(B)]
                s = merge(row_s, parts) * scale
                sbuf[c] = s
                refill(h, c)
                @pl.when(c == TW)
                def _():
                    start_weights(h)
                @pl.when(h == H - 1)
                def _():
                    @pl.when(c == 0)
                    def _():
                        wait_all(wob, wsem.at[3])
                    pl.loop(c * HG, jnp.minimum((c + 1) * HG, H - 1))(project)
                return jnp.maximum(mv, fold(s, jnp.maximum))
            mv = jax.lax.fori_loop(0, NC, kstep, jnp.full((8, 128), -jnp.inf, f32))
            m = jnp.max(mv, axis=-1, keepdims=True)

            @pl.when(h == T_WO)
            def _():
                wait_all(wgb, wsem.at[1])
                wait_all(wub, wsem.at[1])
                wait_all(wdb, wsem.at[2])

            @pl.when(jnp.logical_and(h >= T_WO, h < T_WO + NF))
            def _():
                sl = pl.ds(pl.multiple_of((h - T_WO) * FS, FS), FS)
                x16 = xs[...].astype(bf16)
                g = jnp.dot(x16, wgb[:, sl], preferred_element_type=f32)
                u = jnp.dot(x16, wub[:, sl], preferred_element_type=f32)
                a = (g * jax.nn.sigmoid(g)) * u
                ybuf[...] += jnp.dot(a.astype(bf16), wdb[sl, :], preferred_element_type=f32)

            @pl.when(h == H - 2)
            def _():
                xf = xs[...]
                wr = wrb[...].astype(f32).reshape(1, D)
                r = jnp.sum(xf * wr, axis=-1, keepdims=True)
                ybuf[...] = xf + (xf * 0.0 + ybuf[...] * jax.nn.sigmoid(r))

            def vstep(c, carry):
                lv, o = carry
                slot = (h * NS + NC + c) % S
                p = jnp.exp(sbuf[c] - m)
                lv = lv + fold(p, jnp.add)
                p16 = p.astype(bf16)
                wait_all(ring.at[slot], rsem.at[slot])
                parts = [jnp.dot(p16, ring[slot, b], preferred_element_type=f32) for b in range(B)]
                o = o + merge(row_o, parts)
                refill(h, NC + c)
                return lv, o
            lv, o = jax.lax.fori_loop(0, NC, vstep, (jnp.zeros((8, 128), f32), jnp.zeros((8, Dh), f32)))
            o3[h] = (o / jnp.sum(lv, axis=-1, keepdims=True)).astype(bf16)

        gw = gwb[...].astype(f32).reshape(1, D)
        gate = jax.nn.sigmoid(jnp.sum(xs[...] * gw, axis=-1, keepdims=True))
        jax.lax.fori_loop(0, H, head, None)
        project(H - 1)
        out = gate * abuf[...] + (1.0 - gate) * ybuf[...]
        o_ref[...] = out[0:B, :].astype(o_ref.dtype)

    anyspec = pl.BlockSpec(memory_space=pl.ANY)
    DMA = pltpu.SemaphoreType.DMA
    call = pl.pallas_call(
        kern,
        out_shape=jax.ShapeDtypeStruct((B, D), bf16),
        in_specs=[anyspec] * 10,
        out_specs=pl.BlockSpec(memory_space=pltpu.VMEM),
        scratch_shapes=[
            pltpu.VMEM((S, B, CH, Dh), bf16),
            pltpu.VMEM((D, H * Dh), bf16), pltpu.VMEM((H * Dh, D), bf16),
            pltpu.VMEM((D, F), bf16), pltpu.VMEM((D, F), bf16), pltpu.VMEM((F, D), bf16),
            pltpu.VMEM((B, D), bf16), pltpu.VMEM((D,), bf16), pltpu.VMEM((D,), bf16),
            pltpu.VMEM((8, D), f32), pltpu.VMEM((H, 8, Dh), bf16),
            pltpu.VMEM((NC, 8, CH), f32), pltpu.VMEM((8, D), f32), pltpu.VMEM((8, D), f32),
            DMA((S,)), DMA((4,)), DMA((3,)),
        ],
        compiler_params=pltpu.CompilerParams(vmem_limit_bytes=vmem_mb * 1024 * 1024, disable_bounds_checks=nobc),
    )
    def wrapped(ax, k, v, wq, wo, bx, wr, wg, wu, wd, gw):
        return call(ax.reshape(B, D), k, v, wq, wo, wr, wg, wu, wd, gw).reshape(B, 1, D)
    return wrapped


@jax.jit
def pallas_gated_mix__mha_block_cached__moe_arch_mod__decode_kernel(
    A_x, A_k_cache, A_v_cache, A_wq, A_wo, B_x, B_w_r, B_w_gate, B_w_up, B_w_down, gate_w):
    return build(ORD=1,PART=(192,64),QW=(1024,)*4,FW=(896,)*4,RP=(24,8))(A_x, A_k_cache, A_v_cache, A_wq, A_wo, B_x, B_w_r, B_w_gate, B_w_up, B_w_down, gate_w)
```

```python
import functools

import jax
import jax.experimental.pallas as pl
import jax.experimental.pallas.tpu as pltpu
import jax.numpy as jnp

B, D, H, SK, DH, F = 4, 1024, 32, 8192, 128, 3584

M = 8
G = 4
PIECES = (192, 64)
R = sum(PIECES)
CH = G * R
NC = SK // CH
NS = 2 * NC
SLOTS = 4
NW = 16
FS = 512
NF = F // FS
HG = H // NC

T_WD = D // (8 * 8)
T_WO = T_WD + F // (32 * NW)
T_END = T_WO + H * DH // (32 * NW)
assert T_END < H and T_WO + NF < H and SLOTS <= NC

F32, BF16 = jnp.float32, jnp.bfloat16


def _kernel(x_hbm, k_hbm, v_hbm, wq_hbm, wo_hbm, wr_hbm, wg_hbm, wu_hbm, wd_hbm, gw_hbm,
            out_ref,
            ring, wq, wo, wg, wu, wd, x_in, wr, gw,
            xs, qs, run_max, run_sum, run_pv, heads, scores, y_acc, a_acc,
            ring_sem, w_sem, small_sem):

    def wait_all(buf, sem):
        pltpu.make_async_copy(buf, buf, sem).wait()

    def start_wide(per_queue, c):
        width = per_queue[0][1].shape[1] // 4
        for piece in range(4):
            cols = pl.ds(piece * width, width)
            for stream in range(8):
                for queue, (src, dst, sem, row0, stride) in enumerate(per_queue):
                    rows = pl.ds(pl.multiple_of(row0 + stream * stride + c * 8, 8), 8)
                    pltpu.make_async_copy(
                        src.at[rows, cols], dst.at[rows, cols], sem).start(priority=queue)

    def start_tall(src, dst, sem, c):
        stride = dst.shape[0] // NW
        for r0, size in ((0, 24), (24, 8)):
            for stream in range(8):
                for queue in range(2):
                    row = (stream + 8 * queue) * stride + c * 32 + r0
                    rows = pl.ds(pl.multiple_of(row, 8), size)
                    pltpu.make_async_copy(src.at[rows], dst.at[rows], sem).start(priority=queue)

    def start_kv(src, h, c, slot):
        r0 = 0
        for size in PIECES:
            for b0 in range(B // 2):
                for g in range(G):
                    for queue in range(2):
                        b = b0 + (B // 2) * queue
                        row = pl.multiple_of(g * (SK // G) + c * R + r0, 16)
                        pltpu.make_async_copy(
                            src.at[b, h, pl.ds(row, size)],
                            ring.at[slot, b, pl.ds(g * R + r0, size)],
                            ring_sem.at[slot]).start(priority=queue)
            r0 += size

    def start_step(t):
        h, r, slot = t // NS, t % NS, t % SLOTS

        @pl.when(r < NC)
        def _():
            start_kv(k_hbm, h, r, slot)

        @pl.when(r >= NC)
        def _():
            start_kv(v_hbm, h, r - NC, slot)

    def start_weights(h):
        @pl.when(h < T_WD)
        def _():
            start_wide([(wg_hbm, wg, w_sem.at[1], 0, D // 8),
                        (wu_hbm, wu, w_sem.at[2], 0, D // 8)], h)

        @pl.when(jnp.logical_and(h >= T_WD, h < T_WO))
        def _():
            start_tall(wd_hbm, wd, w_sem.at[3], h - T_WD)

        @pl.when(jnp.logical_and(h >= T_WO, h < T_END))
        def _():
            start_tall(wo_hbm, wo, w_sem.at[4], h - T_WO)

    def fold(a, op):
        return functools.reduce(op, [a[:, i:i + 128] for i in range(0, CH, 128)])

    def per_batch(fn):
        parts = [fn(b) for b in range(B)]
        row = jax.lax.broadcasted_iota(jnp.int32, parts[0].shape, 0)
        merged = jnp.zeros_like(parts[0])
        for b in range(B):
            merged = jnp.where(row == b, parts[b], merged)
        return merged

    def project(h):
        rows = pl.ds(pl.multiple_of(h * DH, DH), DH)
        a_acc[...] += jnp.dot(heads[h], wo[rows, :], preferred_element_type=F32)

    small = [pltpu.make_async_copy(src, dst, small_sem.at[i])
             for i, (src, dst) in enumerate(((x_hbm, x_in), (wr_hbm, wr), (gw_hbm, gw)))]
    for copy in small:
        copy.start()

    @pl.loop(0, D // (8 * NW))
    def _(c):
        start_wide([(wq_hbm, wq, w_sem.at[0], 0, D // NW),
                    (wq_hbm, wq, w_sem.at[0], D // 2, D // NW)], c)

    @pl.loop(0, SLOTS)
    def _(t):
        start_kv(k_hbm, 0, t, t)

    for copy in small:
        copy.wait()

    xs[...] = jnp.zeros(xs.shape, F32)
    xs[0:B, :] = x_in[...].astype(F32)
    y_acc[...] = jnp.zeros(y_acc.shape, F32)
    a_acc[...] = jnp.zeros(a_acc.shape, F32)
    gate = jax.nn.sigmoid(
        jnp.sum(xs[...] * gw[...].astype(F32).reshape(1, D), axis=-1, keepdims=True))
    wait_all(wq, w_sem.at[0])

    @pl.loop(0, H * NS)
    def _(t):
        h, r, slot = t // NS, t % NS, t % SLOTS

        @pl.when(r == 0)
        def _():
            cols = pl.ds(pl.multiple_of(h * DH, DH), DH)
            qs[...] = jnp.dot(xs[...].astype(BF16), wq[:, cols],
                              preferred_element_type=F32).astype(BF16)
            run_max[...] = jnp.full(run_max.shape, -jnp.inf, F32)
            run_sum[...] = jnp.zeros(run_sum.shape, F32)
            run_pv[...] = jnp.zeros(run_pv.shape, F32)

        @pl.when(r < NC)
        def _():
            wait_all(ring.at[slot], ring_sem.at[slot])
            q = qs[...]
            s = per_batch(lambda b: jax.lax.dot_general(
                q, ring[slot, b], (((1,), (1,)), ((), ())),
                preferred_element_type=F32)) * (DH ** -0.5)
            scores[r] = s
            run_max[...] = jnp.maximum(run_max[...], fold(s, jnp.maximum))

        @pl.when(r >= NC)
        def _():
            p = jnp.exp(scores[r - NC] - jnp.max(run_max[...], axis=-1, keepdims=True))
            run_sum[...] += fold(p, jnp.add)
            p16 = p.astype(BF16)
            wait_all(ring.at[slot], ring_sem.at[slot])
            run_pv[...] += per_batch(
                lambda b: jnp.dot(p16, ring[slot, b], preferred_element_type=F32))

        @pl.when(t + SLOTS < H * NS)
        def _():
            start_step(t + SLOTS)

        @pl.when(r == 0)
        def _():
            start_weights(h)

        @pl.when(r == NS - 1)
        def _():
            denom = jnp.sum(run_sum[...], axis=-1, keepdims=True)
            heads[h] = (run_pv[...] / denom).astype(BF16)

        @pl.when(t == T_WO * NS + NC)
        def _():
            wait_all(wg, w_sem.at[1])
            wait_all(wu, w_sem.at[2])
            wait_all(wd, w_sem.at[3])

        @pl.when(jnp.logical_and(r == NC, jnp.logical_and(h >= T_WO, h < T_WO + NF)))
        def _():
            slab = pl.ds(pl.multiple_of((h - T_WO) * FS, FS), FS)
            x16 = xs[...].astype(BF16)
            g = jnp.dot(x16, wg[:, slab], preferred_element_type=F32)
            u = jnp.dot(x16, wu[:, slab], preferred_element_type=F32)
            act = (g * jax.nn.sigmoid(g)) * u
            y_acc[...] += jnp.dot(act.astype(BF16), wd[slab, :], preferred_element_type=F32)

        @pl.when(t == (H - 1) * NS)
        def _():
            x = xs[...]
            router = jnp.sum(x * wr[...].astype(F32).reshape(1, D), axis=-1, keepdims=True)
            y_acc[...] = x + (x * 0.0 + y_acc[...] * jax.nn.sigmoid(router))
            wait_all(wo, w_sem.at[4])

        @pl.when(h == H - 1)
        def _():
            last = r == NS - 1
            lo = jnp.where(last, H - 1, jnp.minimum(r * HG, H - 1))
            hi = jnp.where(last, H, jnp.minimum((r + 1) * HG, H - 1))
            pl.loop(lo, hi)(project)

    out = gate * a_acc[...] + (1.0 - gate) * y_acc[...]
    out_ref[...] = out[0:B, :].astype(out_ref.dtype)


@jax.jit
def pallas_gated_mix__mha_block_cached__moe_arch_mod__decode_kernel(
    A_x: jax.Array,
    A_k_cache: jax.Array,
    A_v_cache: jax.Array,
    A_wq: jax.Array,
    A_wo: jax.Array,
    B_x: jax.Array,
    B_w_r: jax.Array,
    B_w_gate: jax.Array,
    B_w_up: jax.Array,
    B_w_down: jax.Array,
    gate_w: jax.Array,
):
    del B_x
    dma_sem = pltpu.SemaphoreType.DMA
    out = pl.pallas_call(
        _kernel,
        out_shape=jax.ShapeDtypeStruct((B, D), BF16),
        in_specs=[pl.BlockSpec(memory_space=pl.ANY)] * 10,
        out_specs=pl.BlockSpec(memory_space=pltpu.VMEM),
        scratch_shapes=[
            pltpu.VMEM((SLOTS, B, CH, DH), BF16),
            pltpu.VMEM((D, H * DH), BF16),
            pltpu.VMEM((H * DH, D), BF16),
            pltpu.VMEM((D, F), BF16),
            pltpu.VMEM((D, F), BF16),
            pltpu.VMEM((F, D), BF16),
            pltpu.VMEM((B, D), BF16),
            pltpu.VMEM((D,), BF16),
            pltpu.VMEM((D,), BF16),
            pltpu.VMEM((M, D), F32),
            pltpu.VMEM((M, DH), BF16),
            pltpu.VMEM((M, 128), F32),
            pltpu.VMEM((M, 128), F32),
            pltpu.VMEM((M, DH), F32),
            pltpu.VMEM((H, M, DH), BF16),
            pltpu.VMEM((NC, M, CH), F32),
            pltpu.VMEM((M, D), F32),
            pltpu.VMEM((M, D), F32),
            dma_sem((SLOTS,)),
            dma_sem((5,)),
            dma_sem((3,)),
        ],
        compiler_params=pltpu.CompilerParams(vmem_limit_bytes=64 * 1024 * 1024),
    )(A_x.reshape(B, D), A_k_cache, A_v_cache, A_wq, A_wo,
      B_w_r, B_w_gate, B_w_up, B_w_down, gate_w)
    return out.reshape(B, 1, D)
```
